```python
import os as _os
_os.environ.setdefault("JAX_PLATFORMS", "cpu")
import jax
import jax.numpy as jnp

def _softmax(x, axis=-1):
    return jax.nn.softmax(x, axis=axis)
def _gelu(x):
    return jax.nn.gelu(x, approximate=True)
def _silu(x):
    return jax.nn.silu(x)
def _sigmoid(x):
    return jax.nn.sigmoid(x)
def _layernorm(x, axis=-1, eps=1e-5):
    m = jnp.mean(x, axis=axis, keepdims=True)
    v = jnp.var(x, axis=axis, keepdims=True)
    return (x - m) / jnp.sqrt(v + eps)
def _scatter_add(tgt, idx, src, axis=0):
    return tgt.at[idx].add(src)
def _segment_sum(src, seg, n):
    return jax.ops.segment_sum(src, seg, n)
class _Rng:
    def __init__(self, key):
        self._k = key
    def _next(self):
        self._k, sub = jax.random.split(self._k)
        return sub
    def normal(self, shape):
        return jax.random.normal(self._next(), shape, dtype=jnp.bfloat16)
    def randint(self, lo, hi, shape):
        return jax.random.randint(self._next(), shape, lo, hi, dtype=jnp.int32)
    def uniform(self, shape, lo=0.0, hi=1.0):
        return jax.random.uniform(self._next(), shape, jnp.bfloat16, lo, hi)
    def permutation(self, n):
        return jax.random.permutation(self._next(), n)


kernel_name = 'gated_mix__sliding_block_cached__dense_activation_silu__decode'

def setup_inputs():
    _rng = _Rng(jax.random.key(int.from_bytes(__import__("os").urandom(4), "little")))
    _w = (lambda a: (lambda t: t.astype(jnp.bfloat16) if jnp.issubdtype(t.dtype, jnp.floating) else t)(jnp.asarray(a)))
    def _A_setup():
        B, Sq, D = 2, 1, 1024
        Hq, Hkv, Sk, Dh = 32, 4, 32768, 128
        assert Hq % Hkv == 0, (Hq, Hkv)
        return {
            "x": _w((lambda *s: _rng.normal(s) * 0.05)(B, Sq, D)),
            "k_cache": _w((lambda *s: _rng.normal(s) * 3.2)(B, Hkv, Sk, Dh)),
            "v_cache": _w((lambda *s: _rng.normal(s) * 0.05)(B, Hkv, Sk, Dh)),
            "wq": _w((lambda *s: _rng.normal(s) * 3.2)(D, Hq * Dh) * (D ** -0.5)),
            "wo": _w((lambda *s: _rng.normal(s) * 0.05)(Hq * Dh, D) * ((Hq * Dh) ** -0.5)),
        }
    _A_in = _A_setup()

    def _B_setup():
        B, S, D, F = 2, 1, 1024, 3584
        return {
            "x": _w((lambda *s: _rng.normal(s) * 0.05)(B, S, D)),
            "w1": _w((lambda *s: _rng.normal(s) * 0.05)(D, F) * (D ** -0.5)),
            "w2": _w((lambda *s: _rng.normal(s) * 0.05)(F, D) * (F ** -0.5)),
        }
    _B_in = _B_setup()

    return {
        "A_x": _A_in["x"],
        "A_k_cache": _A_in["k_cache"],
        "A_v_cache": _A_in["v_cache"],
        "A_wq": _A_in["wq"],
        "A_wo": _A_in["wo"],
        "B_x": _B_in["x"],
        "B_w1": _B_in["w1"],
        "B_w2": _B_in["w2"],
        "gate_w": _w((lambda *s: _rng.normal(s) * 0.05)(1024) * 16.0),
    }

def reference(A_x, A_k_cache, A_v_cache, A_wq, A_wo, B_x, B_w1, B_w2, gate_w):
    def _A_ref(x, k_cache, v_cache, wq, wo):
        B, Sq, D = x.shape
        Hq, Dh = 32, 128
        Hkv, Sk = k_cache.shape[1], k_cache.shape[2]
        W = min(4096, max(256, Sk // 4))
        rep = Hq // Hkv
        q = (lambda x, *d: x.transpose(*d))((x @ wq).reshape(B, Sq, Hq, Dh), 0, 2, 1, 3)
        k = jnp.repeat(k_cache[:, :, Sk - W:, :], rep, axis=1)
        v = jnp.repeat(v_cache[:, :, Sk - W:, :], rep, axis=1)
        scores = jnp.einsum("bhqd,bhkd->bhqk", q, k) * (Dh ** -0.5)
        p = _softmax(scores, axis=-1)
        o = jnp.einsum("bhqk,bhkd->bhqd", p, v)
        return (lambda x, *d: x.transpose(*d))(o, 0, 2, 1, 3).reshape(B, Sq, Hq * Dh) @ wo

    def _B_ref(x, w1, w2):
        h = jnp.einsum("bsd,df->bsf", x, w1)
        h = _silu(h)
        out = jnp.einsum("bsf,fd->bsd", h, w2)
        return out

    x = A_x
    g = _sigmoid((x * gate_w).sum(-1, keepdims=True))
    a = _A_ref(x, A_k_cache, A_v_cache, A_wq, A_wo)
    b = _B_ref(x, B_w1, B_w2)
    return g * a + (1 - g) * b
```

```python
import functools

import jax
import jax.numpy as jnp
import jax.experimental.pallas as pl
import jax.experimental.pallas.tpu as pltpu

_HQ, _DH = 32, 128
_W2_SPLIT = (1280, 1024, 768, 384, 128)


def _kernel(x_hbm, gw_hbm, k_hbm, v_hbm, wq_hbm, wo_hbm, w1_hbm, w2_hbm, o_ref,
            x_v, gw_v, k_v, v_v, wq_v, wo_v, w1_v, w2_v, p_v, sems, *, w2_split):
    f32, bf16 = jnp.float32, jnp.bfloat16
    B, Hkv, Sk, Dh = k_hbm.shape
    W = k_v.shape[2]
    D = x_v.shape[1]
    rep = _HQ // Hkv
    R = B * rep
    G = rep * Dh

    pairs = [(wq_hbm, wq_v), (x_hbm, x_v), (gw_hbm, gw_v),
             (k_hbm.at[:, :, pl.ds(Sk - W, W), :], k_v),
             (w1_hbm, w1_v),
             (v_hbm.at[:, :, pl.ds(Sk - W, W), :], v_v),
             (wo_hbm, wo_v)]
    offs, off = [], 0
    for n in w2_split:
        pairs.append((w2_hbm.at[pl.ds(off, n), :], w2_v.at[pl.ds(off, n), :]))
        offs.append(off)
        off += n
    cps = [pltpu.make_async_copy(s, d, sems.at[i]) for i, (s, d) in enumerate(pairs)]
    for c in cps:
        c.start()
    c_wq, c_x, c_gw, c_k, c_w1, c_v, c_wo = cps[:7]
    c_w2 = cps[7:]

    c_x.wait()
    c_gw.wait()
    xf = x_v[...].astype(f32)
    gw = gw_v[...].astype(f32).reshape(1, D)
    gate = jax.nn.sigmoid(jnp.sum(xf * gw, axis=-1, keepdims=True))
    xr = jnp.concatenate(
        [jnp.broadcast_to(xf[b:b + 1], (rep, D)) for b in range(B)], axis=0).astype(bf16)
    head = jax.lax.broadcasted_iota(jnp.int32, (R, Dh), 0) % rep

    c_wq.wait()
    qs = []
    for g in range(Hkv):
        qg = jnp.zeros((R, Dh), f32)
        for h in range(rep):
            c0 = (g * rep + h) * Dh
            t = jnp.dot(xr, wq_v[:, c0:c0 + Dh], preferred_element_type=f32)
            qg = jnp.where(head == h, t, qg)
        qs.append(qg)

    c_k.wait()
    inv_l = []
    for g in range(Hkv):
        for b in range(B):
            q = qs[g][b * rep:(b + 1) * rep].astype(bf16)
            s = jax.lax.dot_general(q, k_v[b, g], (((1,), (1,)), ((), ())),
                                    preferred_element_type=f32) * (Dh ** -0.5)
            p = jnp.exp(s - jnp.max(s, axis=-1, keepdims=True))
            inv_l.append(1.0 / jnp.sum(p, axis=-1, keepdims=True))
            p_v[b, g] = p

    c_w1.wait()
    hid = jnp.dot(xr, w1_v[...], preferred_element_type=f32)
    hid = (hid * jax.nn.sigmoid(hid)).astype(bf16)

    c_v.wait()
    os_ = []
    for g in range(Hkv):
        og = jnp.concatenate(
            [jnp.dot(p_v[b, g].astype(bf16), v_v[b, g], preferred_element_type=f32)
             * inv_l[g * B + b] for b in range(B)], axis=0)
        os_.append(jnp.concatenate(
            [jnp.where(head == h, og, 0.0) for h in range(rep)], axis=1).astype(bf16))

    c_wo.wait()
    a = jnp.zeros((R, D), f32)
    for g in range(Hkv):
        a = a + jnp.dot(os_[g], wo_v[g * G:(g + 1) * G, :], preferred_element_type=f32)
    a = jnp.concatenate(
        [jnp.sum(a[b * rep:(b + 1) * rep], axis=0, keepdims=True) for b in range(B)], axis=0)
    a = gate * a

    bb = jnp.zeros((R, D), f32)
    for c, off, n in zip(c_w2, offs, w2_split):
        c.wait()
        bb = bb + jnp.dot(hid[:, off:off + n], w2_v[off:off + n, :],
                          preferred_element_type=f32)
    bb = jnp.concatenate([bb[b * rep:b * rep + 1] for b in range(B)], axis=0)
    o_ref[...] = (a + (1.0 - gate) * bb).astype(o_ref.dtype)


def _build(w2_split=_W2_SPLIT):
    def fn(x, k_cache, v_cache, wq, wo, w1, w2, gate_w):
        B, Hkv, Sk, Dh = k_cache.shape
        D = x.shape[-1]
        W = min(4096, max(256, Sk // 4))
        vm = lambda shape, dt: pltpu.VMEM(shape, dt)
        out = pl.pallas_call(
            functools.partial(_kernel, w2_split=w2_split),
            in_specs=[pl.BlockSpec(memory_space=pltpu.MemorySpace.HBM)] * 8,
            out_shape=jax.ShapeDtypeStruct((B, D), x.dtype),
            scratch_shapes=[
                vm((B, D), x.dtype), vm(gate_w.shape, gate_w.dtype),
                vm((B, Hkv, W, Dh), k_cache.dtype), vm((B, Hkv, W, Dh), v_cache.dtype),
                vm(wq.shape, wq.dtype), vm(wo.shape, wo.dtype),
                vm(w1.shape, w1.dtype), vm(w2.shape, w2.dtype),
                vm((B, Hkv, _HQ // Hkv, W), jnp.float32),
                pltpu.SemaphoreType.DMA((7 + len(w2_split),)),
            ],
            compiler_params=pltpu.CompilerParams(vmem_limit_bytes=100 * 2**20),
        )(x.reshape(B, D), gate_w, k_cache, v_cache, wq, wo, w1, w2)
        return out.reshape(x.shape)
    return fn


@jax.jit
def pallas_gated_mix__sliding_block_cached__dense_activation_silu__decode_kernel(
    A_x: jax.Array,
    A_k_cache: jax.Array,
    A_v_cache: jax.Array,
    A_wq: jax.Array,
    A_wo: jax.Array,
    B_x: jax.Array,
    B_w1: jax.Array,
    B_w2: jax.Array,
    gate_w: jax.Array,
):
    del B_x
    return _build()(A_x, A_k_cache, A_v_cache, A_wq, A_wo, B_w1, B_w2, gate_w)
```
